```python
import jax
import jax.numpy as jnp

def _softmax(x, axis=-1):
    return jax.nn.softmax(x, axis=axis)
def _gelu(x):
    return jax.nn.gelu(x, approximate=True)
def _silu(x):
    return jax.nn.silu(x)
def _sigmoid(x):
    return jax.nn.sigmoid(x)
def _layernorm(x, axis=-1, eps=1e-5):
    m = jnp.mean(x, axis=axis, keepdims=True)
    v = jnp.var(x, axis=axis, keepdims=True)
    return (x - m) / jnp.sqrt(v + eps)
def _scatter_add(tgt, idx, src, axis=0):
    return tgt.at[idx].add(src)
def _segment_sum(src, seg, n):
    return jax.ops.segment_sum(src, seg, n)
class _Rng:
    def __init__(self, key):
        self._k = key
    def _next(self):
        self._k, sub = jax.random.split(self._k)
        return sub
    def normal(self, shape):
        return jax.random.normal(self._next(), shape, dtype=jnp.bfloat16)
    def randint(self, lo, hi, shape):
        return jax.random.randint(self._next(), shape, lo, hi, dtype=jnp.int32)
    def uniform(self, shape, lo=0.0, hi=1.0):
        return jax.random.uniform(self._next(), shape, jnp.bfloat16, lo, hi)
    def permutation(self, n):
        return jax.random.permutation(self._next(), n)


kernel_name = 'interleave_layers__sliding_local_dilated__spectral_gfnet__prompt'

def setup_inputs():
    _rng = _Rng(jax.random.key(int.from_bytes(__import__("os").urandom(4), "little")))
    _w = (lambda a: (lambda t: t.astype(jnp.bfloat16) if jnp.issubdtype(t.dtype, jnp.floating) else t)(jnp.asarray(a)))
    def _A_setup():
        B, S, D = 1, 2048, 1024
        return {
            "x": _w((lambda *s: _rng.normal(s) * 0.05)(B, S, D)),
            "wqkv": _w((lambda *s: _rng.normal(s) * 0.05)(D, 3 * D)),
            "wo": _w((lambda *s: _rng.normal(s) * 0.05)(D, D)),
        }
    _A_in = _A_setup()

    def _B_setup():
        B, S, D = 1, 2048, 1024
        Df = D // 2 + 1
        return {
            "x": _w((lambda *s: _rng.normal(s) * 0.05)(B, S, D)),
            "w_r": _w((lambda *s: _rng.normal(s) * 0.05)(S, Df) * 0.02),
            "w_i": _w((lambda *s: _rng.normal(s) * 0.05)(S, Df) * 0.02),
        }
    _B_in = _B_setup()

    return {
        "A_x": _A_in["x"],
        "A_wqkv": _A_in["wqkv"],
        "A_wo": _A_in["wo"],
        "B_x": _B_in["x"],
        "B_w_r": _B_in["w_r"],
        "B_w_i": _B_in["w_i"],
    }

def reference(A_x, A_wqkv, A_wo, B_x, B_w_r, B_w_i):
    def _A_ref(x, wqkv, wo):
        B, S, D = x.shape
        H = 32; Dh = D // H
        W, dil = 8, 2
        qkv = (lambda x, *d: x.transpose(*d))((x @ wqkv).reshape(B, S, 3, H, Dh), 2, 0, 3, 1, 4)
        q, k, v = qkv[0], qkv[1], qkv[2]
        scale = Dh ** -0.5
        pos = jnp.arange(S)
        off = jnp.arange(W) * dil
        idx = pos[:, None] - off[None, :]
        mask = idx >= 0
        idx_c = jnp.where(mask, idx, 0).reshape(-1)
        kg = k[:, :, idx_c, :].reshape(B, H, S, W, Dh)
        vg = v[:, :, idx_c, :].reshape(B, H, S, W, Dh)
        logits = jnp.einsum("bhsd,bhswd->bhsw", q, kg) * scale
        logits = jnp.where(mask[None, None, :, :], logits, -1e9)
        attn = _softmax(logits, axis=-1)
        o = jnp.einsum("bhsw,bhswd->bhsd", attn, vg)
        return (lambda x, *d: x.transpose(*d))(o, 0, 2, 1, 3).reshape(B, S, D) @ wo

    def _B_ref(x, w_r, w_i):
        B, S, D = x.shape
        X = (lambda x, axes=(-2,-1): jnp.fft.rfft2(x.astype(jnp.float32), axes=axes))(x, axes=(-2, -1))
        W = w_r + 1j * w_i
        X = X * W
        y = (lambda x, s, axes=(-2,-1): jnp.fft.irfft2(x, s=s, axes=axes).astype(jnp.bfloat16))(X, (S, D), axes=(-2, -1))
        return y

    x = A_x
    x = x + _A_ref(_layernorm(x, axis=-1), A_wqkv, A_wo)
    x = x + _B_ref(_layernorm(x, axis=-1), B_w_r, B_w_i)
    x = x + _A_ref(_layernorm(x, axis=-1), A_wqkv, A_wo)
    x = x + _B_ref(_layernorm(x, axis=-1), B_w_r, B_w_i)
    return x
```

```python
import numpy as np
import jax
import jax.numpy as jnp
import jax.experimental.pallas as pl
import jax.experimental.pallas.tpu as pltpu

S, D, H, DH, NW = 2048, 1024, 32, 32, 8
C = 640
T = 256
NT = S // T
BF, F32 = jnp.bfloat16, jnp.float32


def _consts():
    d = np.arange(D)[:, None]
    k = np.arange(512)[None, :]
    ang = 2 * np.pi * ((d * k) % D) / D
    fd = np.concatenate([np.cos(ang), -np.sin(ang)], axis=1)
    fd[:, 512] = (-1.0) ** np.arange(D)
    f0 = np.arange(128)[:, None]
    s0 = np.arange(128)[None, :]
    mf, mi = [], []
    for f1 in range(16):
        a = 2 * np.pi * ((s0 * (16 * f0 + f1)) % S) / S
        r, i = np.cos(a), -np.sin(a)
        m = np.block([[r, -i], [i, r]])
        mf.append(m)
        mi.append(m.T)
    src = np.arange(512).reshape(16, 4, 8).transpose(1, 0, 2).reshape(-1)
    p = np.zeros((512, 512), np.float32)
    p[src, np.arange(512)] = 1
    l = np.arange(128)
    ones = (l[:, None] // 8 == l[None, :] // 8).astype(np.float32)
    return (fd.astype(np.float32), np.stack(mf).astype(np.float32),
            np.stack(mi).astype(np.float32), p, ones)


_FD, _MF, _MI, _P, _ONES = _consts()


def _fft16(xr, xi, sign):
    n = len(xr)
    if n == 1:
        return xr, xi
    er, ei = _fft16(xr[0::2], xi[0::2], sign)
    orr, oi = _fft16(xr[1::2], xi[1::2], sign)
    yr, yi = [None] * n, [None] * n
    for k in range(n // 2):
        if k == 0:
            tr, ti = orr[k], oi[k]
        elif 4 * k == n:
            tr, ti = (-oi[k], orr[k]) if sign > 0 else (oi[k], -orr[k])
        else:
            c = float(np.cos(2 * np.pi * k / n))
            s = float(sign * np.sin(2 * np.pi * k / n))
            tr = orr[k] * c - oi[k] * s
            ti = orr[k] * s + oi[k] * c
        yr[k], yi[k] = er[k] + tr, ei[k] + ti
        yr[k + n // 2], yi[k + n // 2] = er[k] - tr, ei[k] - ti
    return yr, yi


def _ln(x):
    m = jnp.mean(x, axis=-1, keepdims=True)
    xc = x - m
    v = jnp.mean(xc * xc, axis=-1, keepdims=True)
    return (xc * jax.lax.rsqrt(v + 1e-5)).astype(BF)


def _rnd(x):
    return x.astype(BF).astype(F32)


def _dot(a, b):
    return jnp.dot(a, b, preferred_element_type=F32)


def _kernel(x_hbm, wqkv_hbm, wo_hbm, wr_hbm, wi_hbm, fd_hbm, mf_hbm, mi_hbm, p_hbm, ones_hbm,
            o_hbm, xb, wqkv, wo0, wo, wr, wi, fd, mf, mi, p, ones, kv, z, y, wf, sems):
    srcs = [(p_hbm, p), (wqkv_hbm, wqkv), (x_hbm, xb), (ones_hbm, ones), (wo_hbm, wo0),
            (wr_hbm, wr), (wi_hbm, wi), (fd_hbm, fd), (mf_hbm, mf), (mi_hbm, mi)]
    cps = [pltpu.make_async_copy(a, b, sems.at[i]) for i, (a, b) in enumerate(srcs)]
    for c in cps:
        c.start()
    kv[0:16, :] = jnp.zeros((16, 2 * D), F32)
    cps[0].wait()
    cps[1].wait()
    for g in range(6):
        sl = slice(512 * g, 512 * g + 512)
        wqkv[:, sl] = _dot(wqkv[:, sl], p[...]).astype(BF)
    cps[2].wait()
    cps[3].wait()
    cps[4].wait()
    for g in range(2):
        sl = slice(512 * g, 512 * g + 512)
        wo[sl, :] = jax.lax.dot_general(p[...], wo0[sl, :], (((0,), (0,)), ((), ())),
                                        preferred_element_type=F32).astype(BF)

    def layer_a():
        def body(t, _):
            r0 = pl.multiple_of(t * T, T)
            x = xb[pl.ds(r0, T), :].astype(F32)
            h = _ln(x)
            q = _rnd(_dot(h, wqkv[:, 0:D]))
            kv[pl.ds(r0 + 16, T), :] = _rnd(_dot(h, wqkv[:, D:3 * D]))
            win = kv[pl.ds(r0, T + 16), :]
            pos = r0 + jax.lax.broadcasted_iota(jnp.int32, (T, 128), 0)
            outs = []
            for g in range(2):
                prods = []
                for w in range(NW):
                    o = 16 - 2 * w
                    acc = None
                    for j in range(4):
                        c0 = 512 * g + 128 * j
                        pr = q[:, c0:c0 + 128] * win[o:o + T, c0:c0 + 128]
                        acc = pr if acc is None else acc + pr
                    prods.append(acc)
                pc = jnp.concatenate(prods, axis=0)
                hi = pc.astype(BF)
                lo = (pc - hi.astype(F32)).astype(BF)
                lg = (_dot(hi, ones[...]) + _dot(lo, ones[...])) * (DH ** -0.5)
                ls = [lg[0:T]] + [jnp.where(pos >= 2 * w, lg[w * T:(w + 1) * T], -1e9)
                                  for w in range(1, NW)]
                m = ls[0]
                for a in ls[1:]:
                    m = jnp.maximum(m, a)
                es = [jnp.exp(a - m) for a in ls]
                den = es[0]
                for a in es[1:]:
                    den = den + a
                inv = 1.0 / den
                es = [a * inv for a in es]
                for j in range(4):
                    c0 = D + 512 * g + 128 * j
                    acc = None
                    for w in range(NW):
                        o = 16 - 2 * w
                        pr = es[w] * win[o:o + T, c0:c0 + 128]
                        acc = pr if acc is None else acc + pr
                    outs.append(acc.astype(BF))
            ao = jnp.concatenate(outs, axis=1)
            xb[pl.ds(r0, T), :] = (x + _rnd(_dot(ao, wo[...]))).astype(BF)
            return 0
        jax.lax.fori_loop(0, NT, body, 0)

    def radix16(sign):
        def body(i, _):
            r0 = pl.multiple_of(i * 8, 8)
            xr = [z[0, pl.ds(128 * b + r0, 8), :] for b in range(16)]
            xi = [z[1, pl.ds(128 * b + r0, 8), :] for b in range(16)]
            yr, yi = _fft16(xr, xi, sign)
            for b in range(16):
                y[b, 0, pl.ds(r0, 8), :] = yr[b]
                y[b, 1, pl.ds(r0, 8), :] = yi[b]
            return 0
        jax.lax.fori_loop(0, 16, body, 0)

    def layer_b():
        lane0 = jax.lax.broadcasted_iota(jnp.int32, (T, 128), 1) == 0

        def fwd(t, _):
            r0 = pl.multiple_of(t * T, T)
            f = _dot(_ln(xb[pl.ds(r0, T), :].astype(F32)), fd[...])
            rows = pl.ds(r0, T)
            z[0, rows, 0:512] = f[:, 0:512]
            z[0, rows, 512:640] = jnp.where(lane0, f[:, 512:640], 0.0)
            z[1, rows, 0:128] = jnp.where(lane0, 0.0, f[:, 512:640])
            z[1, rows, 128:512] = f[:, 640:1024]
            z[1, rows, 512:640] = jnp.zeros((T, 128), F32)
            return 0
        jax.lax.fori_loop(0, NT, fwd, 0)
        radix16(-1)

        def mid(b, _):
            v = y[b].reshape(256, C).astype(BF)
            s = _dot(mf[b], v)
            sr, si = s[0:128], s[128:256]
            a = jnp.concatenate([wf[0, j, pl.ds(b, 128, stride=16), :] for j in range(5)], axis=1)
            c = jnp.concatenate([wf[1, j, pl.ds(b, 128, stride=16), :] for j in range(5)], axis=1)
            u = jnp.concatenate([sr * a - si * c, sr * c + si * a], axis=0).astype(BF)
            r = _dot(mi[b], u)
            rows = pl.ds(pl.multiple_of(b * 128, 128), 128)
            z[0, rows, :] = r[0:128]
            z[1, rows, :] = r[128:256]
            return 0
        jax.lax.fori_loop(0, 16, mid, 0)
        radix16(1)

        def inv(t, _):
            r0 = pl.multiple_of(t * T, T)
            re = y[pl.ds(2 * t, 2), 0].reshape(T, C)
            im = y[pl.ds(2 * t, 2), 1].reshape(T, C)
            c1 = 1.0 / (S * D)
            u = jnp.concatenate([
                re[:, 0:128] * jnp.where(lane0, c1, 2 * c1), re[:, 128:512] * (2 * c1),
                jnp.where(lane0, re[:, 512:640] * c1, im[:, 0:128] * (2 * c1)),
                im[:, 128:512] * (2 * c1)], axis=1).astype(BF)
            r = jax.lax.dot_general(u, fd[...], (((1,), (1,)), ((), ())),
                                    preferred_element_type=F32)
            xb[pl.ds(r0, T), :] = (xb[pl.ds(r0, T), :].astype(F32) + _rnd(r)).astype(BF)
            return 0
        jax.lax.fori_loop(0, NT, inv, 0)

    layer_a()
    for c in cps[5:]:
        c.wait()
    for i, w in enumerate((wr, wi)):
        for j in range(4):
            wf[i, j] = w[:, 128 * j:128 * j + 128].astype(F32)
        wf[i, 4] = jnp.broadcast_to(w[:, 512:513].astype(F32), (S, 128))
    layer_b()
    layer_a()
    layer_b()
    out = pltpu.make_async_copy(xb, o_hbm, sems.at[0])
    out.start()
    out.wait()


@jax.jit
def pallas_interleave_layers__sliding_local_dilated__spectral_gfnet__prompt_kernel(
    A_x, A_wqkv, A_wo, B_x, B_w_r, B_w_i,
):
    consts = [jnp.asarray(c, dtype=BF) for c in (_FD, _MF, _MI, _P, _ONES)]
    any_spec = pl.BlockSpec(memory_space=pl.ANY)
    vm = pltpu.VMEM
    out = pl.pallas_call(
        _kernel,
        in_specs=[any_spec] * 10,
        out_specs=any_spec,
        out_shape=jax.ShapeDtypeStruct((S, D), BF),
        scratch_shapes=[
            vm((S, D), BF), vm((D, 3 * D), BF), vm((D, D), BF), vm((D, D), BF),
            vm((S, 513), BF), vm((S, 513), BF), vm((D, D), BF),
            vm((16, 256, 256), BF), vm((16, 256, 256), BF), vm((512, 512), BF), vm((128, 128), BF),
            vm((S + 16, 2 * D), F32), vm((2, S, C), F32), vm((16, 2, 128, C), F32),
            vm((2, 5, S, 128), F32), pltpu.SemaphoreType.DMA((10,)),
        ],
        compiler_params=pltpu.CompilerParams(vmem_limit_bytes=120 * 1024 * 1024),
    )(A_x.reshape(S, D), A_wqkv, A_wo, B_w_r, B_w_i, *consts)
    return out.reshape(1, S, D)
```

```python
import numpy as np
import jax
import jax.numpy as jnp
import jax.experimental.pallas as pl
import jax.experimental.pallas.tpu as pltpu

S, D, H, DH, NW = 2048, 1024, 32, 32, 8
C = 640
T = 512
NT = S // T
BF, F32 = jnp.bfloat16, jnp.float32


_PAIRS = ((0, 4), (1, 7), (2, 6), (3, 5))
_RH = float(np.sqrt(0.5))


def _consts():
    d = np.arange(128)[:, None]
    fd = []
    for j, (ka, kb) in enumerate(_PAIRS):
        ca, sa, cb, sb = [f(2 * np.pi * ((d * (8 * np.arange(64)[None, :] + k1)) % D) / D)
                          for k1 in (ka, kb) for f in (np.cos, np.sin)]
        zz = np.zeros_like(ca)
        if j == 0:
            g = np.block([[ca, zz, -sa, zz], [zz, cb, zz, -sb]])
            g[:128, 128] = (-1.0) ** np.arange(128)
        else:
            g = np.block([[ca, cb, -sa, -sb], [sa, -sb, ca, -cb]])
        fd.append(g)
    fd = np.stack(fd)
    f0 = np.arange(128)[:, None]
    s0 = np.arange(128)[None, :]
    mf, mi = [], []
    for f1 in range(16):
        a = 2 * np.pi * ((s0 * (16 * f0 + f1)) % S) / S
        r, i = np.cos(a), -np.sin(a)
        m = np.block([[r, -i], [i, r]])
        mf.append(m)
        mi.append(m.T)
    src = np.arange(512).reshape(16, 4, 8).transpose(1, 0, 2).reshape(-1)
    p = np.zeros((512, 512), np.float32)
    p[src, np.arange(512)] = 1
    l = np.arange(128)
    ones = (l[:, None] // 8 == l[None, :] // 8).astype(np.float32)
    return (fd.astype(np.float32), np.stack(mf).astype(np.float32),
            np.stack(mi).astype(np.float32), p, ones)


_FD, _MF, _MI, _P, _ONES = _consts()


def _fft16(xr, xi, sign):
    n = len(xr)
    if n == 1:
        return xr, xi
    er, ei = _fft16(xr[0::2], xi[0::2], sign)
    orr, oi = _fft16(xr[1::2], xi[1::2], sign)
    yr, yi = [None] * n, [None] * n
    for k in range(n // 2):
        if k == 0:
            tr, ti = orr[k], oi[k]
        elif 4 * k == n:
            tr, ti = (-oi[k], orr[k]) if sign > 0 else (oi[k], -orr[k])
        else:
            c = float(np.cos(2 * np.pi * k / n))
            s = float(sign * np.sin(2 * np.pi * k / n))
            tr = orr[k] * c - oi[k] * s
            ti = orr[k] * s + oi[k] * c
        yr[k], yi[k] = er[k] + tr, ei[k] + ti
        yr[k + n // 2], yi[k + n // 2] = er[k] - tr, ei[k] - ti
    return yr, yi


def _ln(x):
    m = jnp.mean(x, axis=-1, keepdims=True)
    xc = x - m
    v = jnp.mean(xc * xc, axis=-1, keepdims=True)
    return (xc * jax.lax.rsqrt(v + 1e-5)).astype(BF)


def _rnd(x):
    return x.astype(BF).astype(F32)


def _dot(a, b):
    return jnp.dot(a, b, preferred_element_type=F32)


def _kernel(x_hbm, wqkv_hbm, wo_hbm, wr_hbm, wi_hbm, fd_hbm, mf_hbm, mi_hbm, p_hbm, ones_hbm,
            o_hbm, xb, wqkv, wo0, wo, wr, wi, fd, mf, mi, p, ones, kv, z, y, wf, wt, sems):
    srcs = [(p_hbm, p), (wqkv_hbm, wqkv), (x_hbm, xb), (ones_hbm, ones), (wo_hbm, wo0),
            (wr_hbm, wr), (wi_hbm, wi), (fd_hbm, fd), (mf_hbm, mf), (mi_hbm, mi)]
    cps = [pltpu.make_async_copy(a, b, sems.at[i]) for i, (a, b) in enumerate(srcs)]
    cps[0].start()
    cps[1].start()
    kv[0:16, :] = jnp.zeros((16, 2 * D), F32)
    cps[0].wait()
    cps[1].wait()
    for c in cps[2:]:
        c.start()
    for g in range(6):
        sl = slice(512 * g, 512 * g + 512)
        wqkv[:, sl] = _dot(wqkv[:, sl], p[...]).astype(BF)
    cps[2].wait()
    cps[3].wait()
    cps[4].wait()
    for g in range(2):
        sl = slice(512 * g, 512 * g + 512)
        wo[sl, :] = jax.lax.dot_general(p[...], wo0[sl, :], (((0,), (0,)), ((), ())),
                                        preferred_element_type=F32).astype(BF)

    def layer_a():
        def body(t, _):
            r0 = pl.multiple_of(t * T, T)
            x = xb[pl.ds(r0, T), :].astype(F32)
            h = _ln(x)
            q = _rnd(_dot(h, wqkv[:, 0:D]))
            kv[pl.ds(r0 + 16, T), :] = _rnd(_dot(h, wqkv[:, D:3 * D]))
            win = kv[pl.ds(r0, T + 16), :]
            rot = [win[8 - 2 * r:16 - 2 * r + T] for r in range(4)]

            def sh(w, c0):
                o = 8 - 8 * (w // 4)
                return rot[w % 4][o:o + T, c0:c0 + 128]

            pos = r0 + jax.lax.broadcasted_iota(jnp.int32, (T, 128), 0)
            outs = []
            for g in range(2):
                prods = []
                for w in range(NW):
                    o = 16 - 2 * w
                    acc = None
                    for j in range(4):
                        c0 = 512 * g + 128 * j
                        pr = q[:, c0:c0 + 128] * sh(w, c0)
                        acc = pr if acc is None else acc + pr
                    prods.append(acc)
                pc = jnp.concatenate(prods, axis=0)
                hi = pc.astype(BF)
                lo = (pc - hi.astype(F32)).astype(BF)
                lg = (_dot(hi, ones[...]) + _dot(lo, ones[...])) * (DH ** -0.5)
                ls = [lg[0:T]] + [jnp.where(pos >= 2 * w, lg[w * T:(w + 1) * T], -1e9)
                                  for w in range(1, NW)]
                m = ls[0]
                for a in ls[1:]:
                    m = jnp.maximum(m, a)
                es = [jnp.exp(a - m) for a in ls]
                den = es[0]
                for a in es[1:]:
                    den = den + a
                inv = 1.0 / den
                es = [a * inv for a in es]
                for j in range(4):
                    c0 = D + 512 * g + 128 * j
                    acc = None
                    for w in range(NW):
                        o = 16 - 2 * w
                        pr = es[w] * sh(w, c0)
                        acc = pr if acc is None else acc + pr
                    outs.append(acc.astype(BF))
            ao = jnp.concatenate(outs, axis=1)
            xb[pl.ds(r0, T), :] = (x + _rnd(_dot(ao, wo[...]))).astype(BF)
            return 0
        jax.lax.fori_loop(0, NT, body, 0)

    def radix16(sign):
        def r16(i, _):
            r0 = pl.multiple_of(i * 8, 8)
            xr = [z[0, pl.ds(128 * b + r0, 8), :] for b in range(16)]
            xi = [z[1, pl.ds(128 * b + r0, 8), :] for b in range(16)]
            yr, yi = _fft16(xr, xi, sign)
            for b in range(16):
                y[b, 0, pl.ds(r0, 8), :] = yr[b]
                y[b, 1, pl.ds(r0, 8), :] = yi[b]
            return 0
        jax.lax.fori_loop(0, 16, r16, 0)

    def layer_b():
        lane0 = jax.lax.broadcasted_iota(jnp.int32, (T, 128), 1) == 0

        def fwd(t, _):
            r0 = pl.multiple_of(t * T, T)
            h = _ln(xb[pl.ds(r0, T), :].astype(F32)).astype(F32)
            rows = pl.ds(r0, T)
            x = [h[:, 128 * i:128 * i + 128] for i in range(8)]
            sm = [x[i] + x[i + 4] for i in range(4)]
            df = [x[i] - x[i + 4] for i in range(4)]
            e, o = sm[0] + sm[2], sm[1] + sm[3]
            pp, qq = (df[1] - df[3]) * _RH, (df[1] + df[3]) * _RH
            ys = [(e + o, e - o), (df[0] + pp, -df[2] - qq),
                  (sm[0] - sm[2], sm[3] - sm[1]), (df[0] - pp, df[2] - qq)]
            for j in range(4):
                f = _dot(jnp.concatenate(ys[j], axis=1).astype(BF), fd[j])
                fi = f[:, 128:256]
                if j == 0:
                    z[0, rows, 512:640] = jnp.where(lane0, fi, 0.0)
                    fi = jnp.where(lane0, 0.0, fi)
                z[0, rows, 128 * j:128 * j + 128] = f[:, 0:128]
                z[1, rows, 128 * j:128 * j + 128] = fi
            z[1, rows, 512:640] = jnp.zeros((T, 128), F32)
            return 0
        jax.lax.fori_loop(0, NT, fwd, 0)
        radix16(-1)

        def mid(b, _):
            v = y[b].reshape(256, C).astype(BF)
            s = _dot(mf[b], v)
            sr, si = s[0:128], s[128:256]
            a = jnp.concatenate([wf[0, j, pl.ds(b, 128, stride=16), :] for j in range(5)], axis=1)
            c = jnp.concatenate([wf[1, j, pl.ds(b, 128, stride=16), :] for j in range(5)], axis=1)
            u = jnp.concatenate([sr * a - si * c, sr * c + si * a], axis=0).astype(BF)
            r = _dot(mi[b], u)
            rows = pl.ds(pl.multiple_of(b * 128, 128), 128)
            z[0, rows, :] = r[0:128]
            z[1, rows, :] = r[128:256]
            return 0
        jax.lax.fori_loop(0, 16, mid, 0)
        radix16(1)

        def inv(t, _):
            r0 = pl.multiple_of(t * T, T)
            re = y[pl.ds(4 * t, 4), 0].reshape(T, C)
            im = y[pl.ds(4 * t, 4), 1].reshape(T, C)
            c1 = 1.0 / (S * D)
            g = []
            for j in range(4):
                ur, ui = re[:, 128 * j:128 * j + 128], im[:, 128 * j:128 * j + 128]
                if j == 0:
                    ur = ur * jnp.where(lane0, 0.5, 1.0)
                    ui = jnp.where(lane0, re[:, 512:640] * 0.5, ui)
                u = jnp.concatenate([ur, ui], axis=1).astype(BF)
                r = jax.lax.dot_general(u, fd[j], (((1,), (1,)), ((), ())),
                                        preferred_element_type=F32) * (2 * c1)
                g.append((r[:, 0:128], r[:, 128:256]))
            e, o = g[0][0] + g[0][1], g[0][0] - g[0][1]
            sm = [e + g[2][0], o - g[2][1], e - g[2][0], o + g[2][1]]
            pp, qq = (g[1][0] - g[3][0]) * _RH, (g[1][1] + g[3][1]) * _RH
            df = [g[1][0] + g[3][0], pp - qq, g[3][1] - g[1][1], -pp - qq]
            r = jnp.concatenate([sm[i] + df[i] for i in range(4)]
                                + [sm[i] - df[i] for i in range(4)], axis=1)
            xb[pl.ds(r0, T), :] = (xb[pl.ds(r0, T), :].astype(F32) + _rnd(r)).astype(BF)
            return 0
        jax.lax.fori_loop(0, NT, inv, 0)

    layer_a()
    for c in cps[5:]:
        c.wait()
    for i, w in enumerate((wr, wi)):
        for t in range(16):
            cs = slice(128 * t, 128 * t + 128)
            wt[...] = w[0:512, cs].astype(F32)
            for j, (ka, kb) in enumerate(_PAIRS):
                blk = jnp.concatenate([wt[pl.ds(ka, 64, stride=8), :],
                                       wt[pl.ds(kb, 64, stride=8), :]], axis=0)
                wf[i, j, cs, :] = blk.T
            wf[i, 4, cs, :] = jnp.broadcast_to(w[512:513, cs].astype(F32), (128, 128)).T
    layer_b()
    layer_a()
    layer_b()
    out = pltpu.make_async_copy(xb, o_hbm, sems.at[0])
    out.start()
    out.wait()


@jax.jit
def pallas_interleave_layers__sliding_local_dilated__spectral_gfnet__prompt_kernel(
    A_x, A_wqkv, A_wo, B_x, B_w_r, B_w_i,
):
    consts = [jnp.asarray(c, dtype=BF) for c in (_FD, _MF, _MI, _P, _ONES)]
    any_spec = pl.BlockSpec(memory_space=pl.ANY)
    vm = pltpu.VMEM
    out = pl.pallas_call(
        _kernel,
        in_specs=[any_spec] * 10,
        out_specs=any_spec,
        out_shape=jax.ShapeDtypeStruct((S, D), BF),
        scratch_shapes=[
            vm((S, D), BF), vm((D, 3 * D), BF), vm((D, D), BF), vm((D, D), BF),
            vm((513, S), BF), vm((513, S), BF), vm((4, 256, 256), BF),
            vm((16, 256, 256), BF), vm((16, 256, 256), BF), vm((512, 512), BF), vm((128, 128), BF),
            vm((S + 16, 2 * D), F32), vm((2, S, C), F32), vm((16, 2, 128, C), F32),
            vm((2, 5, S, 128), F32), vm((512, 128), F32), pltpu.SemaphoreType.DMA((10,)),
        ],
        compiler_params=pltpu.CompilerParams(vmem_limit_bytes=120 * 1024 * 1024),
    )(A_x.reshape(S, D), A_wqkv, A_wo, B_w_r.T, B_w_i.T, *consts)
    return out.reshape(1, S, D)
```

```python
import numpy as np
import jax
import jax.numpy as jnp
import jax.experimental.pallas as pl
import jax.experimental.pallas.tpu as pltpu

S, D, H, DH, NW = 2048, 1024, 32, 32, 8
C = 640
T = 256
NT = S // T
BF, F32 = jnp.bfloat16, jnp.float32


_PAIRS = ((0, 4), (1, 7), (2, 6), (3, 5))
_RH = float(np.sqrt(0.5))


def _consts():
    d = np.arange(128)[:, None]
    fd = []
    for j, (ka, kb) in enumerate(_PAIRS):
        ca, sa, cb, sb = [f(2 * np.pi * ((d * (8 * np.arange(64)[None, :] + k1)) % D) / D)
                          for k1 in (ka, kb) for f in (np.cos, np.sin)]
        zz = np.zeros_like(ca)
        if j == 0:
            g = np.block([[ca, zz, -sa, zz], [zz, cb, zz, -sb]])
            g[:128, 128] = (-1.0) ** np.arange(128)
        else:
            g = np.block([[ca, cb, -sa, -sb], [sa, -sb, ca, -cb]])
        fd.append(g)
    fd = np.stack(fd)
    f0 = np.arange(128)[:, None]
    s0 = np.arange(128)[None, :]
    mf, mi = [], []
    for f1 in range(16):
        a = 2 * np.pi * ((s0 * (16 * f0 + f1)) % S) / S
        r, i = np.cos(a), -np.sin(a)
        m = np.block([[r, -i], [i, r]])
        mf.append(m)
        mi.append(m.T)
    src = np.arange(512).reshape(16, 4, 8).transpose(1, 0, 2).reshape(-1)
    p = np.zeros((512, 512), np.float32)
    p[src, np.arange(512)] = 1
    l = np.arange(128)
    ones = (l[:, None] // 8 == l[None, :] // 8).astype(np.float32)
    return (fd.astype(np.float32), np.stack(mf).astype(np.float32),
            np.stack(mi).astype(np.float32), p, ones)


_FD, _MF, _MI, _P, _ONES = _consts()


def _fft16(xr, xi, sign):
    n = len(xr)
    if n == 1:
        return xr, xi
    er, ei = _fft16(xr[0::2], xi[0::2], sign)
    orr, oi = _fft16(xr[1::2], xi[1::2], sign)
    yr, yi = [None] * n, [None] * n
    for k in range(n // 2):
        if k == 0:
            tr, ti = orr[k], oi[k]
        elif 4 * k == n:
            tr, ti = (-oi[k], orr[k]) if sign > 0 else (oi[k], -orr[k])
        else:
            c = float(np.cos(2 * np.pi * k / n))
            s = float(sign * np.sin(2 * np.pi * k / n))
            tr = orr[k] * c - oi[k] * s
            ti = orr[k] * s + oi[k] * c
        yr[k], yi[k] = er[k] + tr, ei[k] + ti
        yr[k + n // 2], yi[k + n // 2] = er[k] - tr, ei[k] - ti
    return yr, yi


def _ln(x):
    m = jnp.mean(x, axis=-1, keepdims=True)
    xc = x - m
    v = jnp.mean(xc * xc, axis=-1, keepdims=True)
    return (xc * jax.lax.rsqrt(v + 1e-5)).astype(BF)


def _rnd(x):
    return x.astype(BF).astype(F32)


def _dot(a, b):
    return jnp.dot(a, b, preferred_element_type=F32)


def _kernel(x_hbm, wqkv_hbm, wo_hbm, wr_hbm, wi_hbm, fd_hbm, mf_hbm, mi_hbm, p_hbm, ones_hbm,
            o_hbm, xb, wqkv, wo0, wo, wr, wi, fd, mf, mi, p, ones, kv, z, y, wf, wt, sems):
    srcs = [(p_hbm, p), (wqkv_hbm, wqkv), (x_hbm, xb), (ones_hbm, ones), (wo_hbm, wo0),
            (wr_hbm, wr), (wi_hbm, wi), (fd_hbm, fd), (mf_hbm, mf), (mi_hbm, mi)]
    cps = [pltpu.make_async_copy(a, b, sems.at[i]) if i != 1 else None
           for i, (a, b) in enumerate(srcs)]
    cps[0].start()
    wch = [pltpu.make_async_copy(wqkv_hbm.at[pl.ds(256 * g, 256)], wqkv.at[pl.ds(256 * g, 256)],
                                 sems.at[10 + g]) for g in range(4)]
    for c in wch:
        c.start()
    kv[0:16, :] = jnp.zeros((16, 2 * D), F32)
    cps[0].wait()
    for c in cps[2:]:
        c.start()
    for r in range(4):
        wch[r].wait()
        for g in range(6):
            rs, sl = slice(256 * r, 256 * r + 256), slice(512 * g, 512 * g + 512)
            wqkv[rs, sl] = _dot(wqkv[rs, sl], p[...]).astype(BF)
    cps[2].wait()
    cps[3].wait()
    cps[4].wait()
    for g in range(2):
        sl = slice(512 * g, 512 * g + 512)
        wo[sl, :] = jax.lax.dot_general(p[...], wo0[sl, :], (((0,), (0,)), ((), ())),
                                        preferred_element_type=F32).astype(BF)

    def layer_a():
        def body(t, _):
            r0 = pl.multiple_of(t * T, T)
            x = xb[pl.ds(r0, T), :].astype(F32)
            h = _ln(x)
            q = _dot(h, wqkv[:, 0:D]) * (DH ** -0.5)
            kv[pl.ds(r0 + 16, T), :] = _dot(h, wqkv[:, D:3 * D])
            win = kv[pl.ds(r0, T + 16), :]
            rot = [win[8 - 2 * r:16 - 2 * r + T] for r in range(4)]

            def sh(w, c0):
                o = 8 - 8 * (w // 4)
                return rot[w % 4][o:o + T, c0:c0 + 128]

            pos = r0 + jax.lax.broadcasted_iota(jnp.int32, (T, 128), 0)
            outs = []
            for g in range(2):
                prods = []
                for w in range(NW):
                    o = 16 - 2 * w
                    acc = None
                    for j in range(4):
                        c0 = 512 * g + 128 * j
                        pr = q[:, c0:c0 + 128] * sh(w, c0)
                        acc = pr if acc is None else acc + pr
                    prods.append(acc)
                pc = jnp.concatenate(prods, axis=0)
                hi = pc.astype(BF)
                lg = _dot(hi, ones[...])
                ls = [lg[0:T]] + [jnp.where(pos >= 2 * w, lg[w * T:(w + 1) * T], -1e9)
                                  for w in range(1, NW)]
                m = ls[0]
                for a in ls[1:]:
                    m = jnp.maximum(m, a)
                es = [jnp.exp(a - m) for a in ls]
                den = es[0]
                for a in es[1:]:
                    den = den + a
                inv = 1.0 / den
                es = [a * inv for a in es]
                for j in range(4):
                    c0 = D + 512 * g + 128 * j
                    acc = None
                    for w in range(NW):
                        o = 16 - 2 * w
                        pr = es[w] * sh(w, c0)
                        acc = pr if acc is None else acc + pr
                    outs.append(acc.astype(BF))
            ao = jnp.concatenate(outs, axis=1)
            xb[pl.ds(r0, T), :] = (x + _rnd(_dot(ao, wo[...]))).astype(BF)
            return 0
        jax.lax.fori_loop(0, NT, body, 0)

    def radix16(sign):
        def r16(i, _):
            r0 = pl.multiple_of(i * 8, 8)
            xr = [z[0, pl.ds(128 * b + r0, 8), :] for b in range(16)]
            xi = [z[1, pl.ds(128 * b + r0, 8), :] for b in range(16)]
            yr, yi = _fft16(xr, xi, sign)
            for b in range(16):
                y[b, 0, pl.ds(r0, 8), :] = yr[b]
                y[b, 1, pl.ds(r0, 8), :] = yi[b]
            return 0
        jax.lax.fori_loop(0, 16, r16, 0)

    def layer_b():
        lane0 = jax.lax.broadcasted_iota(jnp.int32, (T, 128), 1) == 0

        def fwd(t, _):
            r0 = pl.multiple_of(t * T, T)
            h = _ln(xb[pl.ds(r0, T), :].astype(F32)).astype(F32)
            rows = pl.ds(r0, T)
            x = [h[:, 128 * i:128 * i + 128] for i in range(8)]
            sm = [x[i] + x[i + 4] for i in range(4)]
            df = [x[i] - x[i + 4] for i in range(4)]
            e, o = sm[0] + sm[2], sm[1] + sm[3]
            pp, qq = (df[1] - df[3]) * _RH, (df[1] + df[3]) * _RH
            ys = [(e + o, e - o), (df[0] + pp, -df[2] - qq),
                  (sm[0] - sm[2], sm[3] - sm[1]), (df[0] - pp, df[2] - qq)]
            for j in range(4):
                f = _dot(jnp.concatenate(ys[j], axis=1).astype(BF), fd[j])
                fi = f[:, 128:256]
                if j == 0:
                    z[0, rows, 512:640] = jnp.where(lane0, fi, 0.0)
                    fi = jnp.where(lane0, 0.0, fi)
                z[0, rows, 128 * j:128 * j + 128] = f[:, 0:128]
                z[1, rows, 128 * j:128 * j + 128] = fi
            z[1, rows, 512:640] = jnp.zeros((T, 128), F32)
            return 0
        jax.lax.fori_loop(0, NT, fwd, 0)
        radix16(-1)

        def mid(b, _):
            v = y[b].reshape(256, C).astype(BF)
            s = _dot(mf[b], v)
            sr, si = s[0:128], s[128:256]
            a = jnp.concatenate([wf[0, j, pl.ds(b, 128, stride=16), :] for j in range(5)], axis=1)
            c = jnp.concatenate([wf[1, j, pl.ds(b, 128, stride=16), :] for j in range(5)], axis=1)
            u = jnp.concatenate([sr * a - si * c, sr * c + si * a], axis=0).astype(BF)
            r = _dot(mi[b], u)
            rows = pl.ds(pl.multiple_of(b * 128, 128), 128)
            z[0, rows, :] = r[0:128]
            z[1, rows, :] = r[128:256]
            return 0
        jax.lax.fori_loop(0, 16, mid, 0, unroll=2)
        radix16(1)

        def inv(t, _):
            r0 = pl.multiple_of(t * T, T)
            re = y[pl.ds(2 * t, 2), 0].reshape(T, C)
            im = y[pl.ds(2 * t, 2), 1].reshape(T, C)
            c1 = 1.0 / (S * D)
            g = []
            for j in range(4):
                ur, ui = re[:, 128 * j:128 * j + 128], im[:, 128 * j:128 * j + 128]
                if j == 0:
                    ur = ur * jnp.where(lane0, 0.5, 1.0)
                    ui = jnp.where(lane0, re[:, 512:640] * 0.5, ui)
                u = jnp.concatenate([ur, ui], axis=1).astype(BF)
                r = jax.lax.dot_general(u, fd[j], (((1,), (1,)), ((), ())),
                                        preferred_element_type=F32) * (2 * c1)
                g.append((r[:, 0:128], r[:, 128:256]))
            e, o = g[0][0] + g[0][1], g[0][0] - g[0][1]
            sm = [e + g[2][0], o - g[2][1], e - g[2][0], o + g[2][1]]
            pp, qq = (g[1][0] - g[3][0]) * _RH, (g[1][1] + g[3][1]) * _RH
            df = [g[1][0] + g[3][0], pp - qq, g[3][1] - g[1][1], -pp - qq]
            r = jnp.concatenate([sm[i] + df[i] for i in range(4)]
                                + [sm[i] - df[i] for i in range(4)], axis=1)
            xb[pl.ds(r0, T), :] = (xb[pl.ds(r0, T), :].astype(F32) + _rnd(r)).astype(BF)
            return 0
        jax.lax.fori_loop(0, NT, inv, 0)

    layer_a()
    for c in cps[5:]:
        c.wait()
    for i, w in enumerate((wr, wi)):
        for t in range(16):
            cs = slice(128 * t, 128 * t + 128)
            wt[...] = w[0:512, cs].astype(F32)
            for j, (ka, kb) in enumerate(_PAIRS):
                blk = jnp.concatenate([wt[pl.ds(ka, 64, stride=8), :],
                                       wt[pl.ds(kb, 64, stride=8), :]], axis=0)
                wf[i, j, cs, :] = blk.T
            wf[i, 4, cs, :] = jnp.broadcast_to(w[512:513, cs].astype(F32), (128, 128)).T
    layer_b()
    layer_a()
    layer_b()
    out = pltpu.make_async_copy(xb, o_hbm, sems.at[0])
    out.start()
    out.wait()


@jax.jit
def pallas_interleave_layers__sliding_local_dilated__spectral_gfnet__prompt_kernel(
    A_x, A_wqkv, A_wo, B_x, B_w_r, B_w_i,
):
    consts = [jnp.asarray(c, dtype=BF) for c in (_FD, _MF, _MI, _P, _ONES)]
    any_spec = pl.BlockSpec(memory_space=pl.ANY)
    vm = pltpu.VMEM
    out = pl.pallas_call(
        _kernel,
        in_specs=[any_spec] * 10,
        out_specs=any_spec,
        out_shape=jax.ShapeDtypeStruct((S, D), BF),
        scratch_shapes=[
            vm((S, D), BF), vm((D, 3 * D), BF), vm((D, D), BF), vm((D, D), BF),
            vm((513, S), BF), vm((513, S), BF), vm((4, 256, 256), BF),
            vm((16, 256, 256), BF), vm((16, 256, 256), BF), vm((512, 512), BF), vm((128, 128), BF),
            vm((S + 16, 2 * D), F32), vm((2, S, C), F32), vm((16, 2, 128, C), F32),
            vm((2, 5, S, 128), F32), vm((512, 128), F32), pltpu.SemaphoreType.DMA((14,)),
        ],
        compiler_params=pltpu.CompilerParams(vmem_limit_bytes=120 * 1024 * 1024),
    )(A_x.reshape(S, D), A_wqkv, A_wo, B_w_r.T, B_w_i.T, *consts)
    return out.reshape(1, S, D)
```
